```python
import os as _os
_os.environ.setdefault("JAX_PLATFORMS", "cpu")
import jax
import jax.numpy as jnp

def _softmax(x, axis=-1):
    return jax.nn.softmax(x, axis=axis)
def _gelu(x):
    return jax.nn.gelu(x, approximate=True)
def _silu(x):
    return jax.nn.silu(x)
def _sigmoid(x):
    return jax.nn.sigmoid(x)
def _layernorm(x, axis=-1, eps=1e-5):
    m = jnp.mean(x, axis=axis, keepdims=True)
    v = jnp.var(x, axis=axis, keepdims=True)
    return (x - m) / jnp.sqrt(v + eps)
def _scatter_add(tgt, idx, src, axis=0):
    return tgt.at[idx].add(src)
def _segment_sum(src, seg, n):
    return jax.ops.segment_sum(src, seg, n)
class _Rng:
    def __init__(self, key):
        self._k = key
    def _next(self):
        self._k, sub = jax.random.split(self._k)
        return sub
    def normal(self, shape):
        return jax.random.normal(self._next(), shape, dtype=jnp.bfloat16)
    def randint(self, lo, hi, shape):
        return jax.random.randint(self._next(), shape, lo, hi, dtype=jnp.int32)
    def uniform(self, shape, lo=0.0, hi=1.0):
        return jax.random.uniform(self._next(), shape, jnp.bfloat16, lo, hi)
    def permutation(self, n):
        return jax.random.permutation(self._next(), n)


kernel_name = 'concat_heads__mha_block_cached__mha_block_cached__near_ridge'

def setup_inputs():
    _rng = _Rng(jax.random.key(int.from_bytes(__import__("os").urandom(4), "little")))
    _w = (lambda a: (lambda t: t.astype(jnp.bfloat16) if jnp.issubdtype(t.dtype, jnp.floating) else t)(jnp.asarray(a)))
    def _A_setup():
        B, Sq, D = 8, 144, 640
        H, Sk, Dh = 32, 512, 128
        return {
            "x": _w((lambda *s: _rng.normal(s) * 0.8)(B, Sq, D)),
            "k_cache": _w((lambda *s: _rng.normal(s) * 0.8)(B, H, Sk, Dh)),
            "v_cache": _w((lambda *s: _rng.normal(s) * 0.05)(B, H, Sk, Dh)),
            "wq": _w((lambda *s: _rng.normal(s) * 0.8)(D, H * Dh) * (D ** -0.5)),
            "wo": _w((lambda *s: _rng.normal(s) * 0.05)(H * Dh, D) * ((H * Dh) ** -0.5)),
        }
    _A_in = _A_setup()

    def _B_setup():
        B, Sq, D = 8, 144, 640
        H, Sk, Dh = 32, 512, 128
        return {
            "x": _w((lambda *s: _rng.normal(s) * 0.8)(B, Sq, D)),
            "k_cache": _w((lambda *s: _rng.normal(s) * 0.8)(B, H, Sk, Dh)),
            "v_cache": _w((lambda *s: _rng.normal(s) * 0.05)(B, H, Sk, Dh)),
            "wq": _w((lambda *s: _rng.normal(s) * 0.8)(D, H * Dh) * (D ** -0.5)),
            "wo": _w((lambda *s: _rng.normal(s) * 0.05)(H * Dh, D) * ((H * Dh) ** -0.5)),
        }
    _B_in = _B_setup()

    return {
        "A_x": _A_in["x"],
        "A_k_cache": _A_in["k_cache"],
        "A_v_cache": _A_in["v_cache"],
        "A_wq": _A_in["wq"],
        "A_wo": _A_in["wo"],
        "B_x": _B_in["x"],
        "B_k_cache": _B_in["k_cache"],
        "B_v_cache": _B_in["v_cache"],
        "B_wq": _B_in["wq"],
        "B_wo": _B_in["wo"],
    }

def reference(A_x, A_k_cache, A_v_cache, A_wq, A_wo, B_x, B_k_cache, B_v_cache, B_wq, B_wo):
    def _A_ref(x, k_cache, v_cache, wq, wo):
        B, Sq, D = x.shape
        H, Dh = 32, 128
        q = (lambda x, *d: x.transpose(*d))((x @ wq).reshape(B, Sq, H, Dh), 0, 2, 1, 3)
        scores = jnp.einsum("bhqd,bhkd->bhqk", q, k_cache) * (Dh ** -0.5)
        p = _softmax(scores, axis=-1)
        o = jnp.einsum("bhqk,bhkd->bhqd", p, v_cache)
        return (lambda x, *d: x.transpose(*d))(o, 0, 2, 1, 3).reshape(B, Sq, H * Dh) @ wo

    def _B_ref(x, k_cache, v_cache, wq, wo):
        B, Sq, D = x.shape
        H, Dh = 32, 128
        q = (lambda x, *d: x.transpose(*d))((x @ wq).reshape(B, Sq, H, Dh), 0, 2, 1, 3)
        scores = jnp.einsum("bhqd,bhkd->bhqk", q, k_cache) * (Dh ** -0.5)
        p = _softmax(scores, axis=-1)
        o = jnp.einsum("bhqk,bhkd->bhqd", p, v_cache)
        return (lambda x, *d: x.transpose(*d))(o, 0, 2, 1, 3).reshape(B, Sq, H * Dh) @ wo

    a = _A_ref(A_x, A_k_cache, A_v_cache, A_wq, A_wo)
    b = _B_ref(B_x, B_k_cache, B_v_cache, B_wq, B_wo)
    return jnp.concatenate([a, b], axis=-1)
```

```python
import math

import jax
import jax.numpy as jnp
from jax import lax
import jax.experimental.pallas as pl
import jax.experimental.pallas.tpu as pltpu

B, SQ, D = 8, 144, 640
H, SK, DH = 32, 512, 128
HD = H * DH
NBLK = 2
NITEMS = NBLK * B
NB = 4

Q_SCALE = (DH ** -0.5) * math.log2(math.e)


def _qk(q, k):
    return lax.dot_general(q, k, (((1,), (1,)), ((), ())),
                           preferred_element_type=jnp.float32)


def _softmax_pv(s, v):
    m = jnp.max(s, axis=-1, keepdims=True)
    p = jnp.exp2(s - m)
    l = jnp.sum(p, axis=-1, keepdims=True)
    o = jnp.dot(p.astype(jnp.bfloat16), v, preferred_element_type=jnp.float32)
    return (o * (1.0 / l)).astype(jnp.bfloat16)


def _kernel(xa, ka, va, wqa, woa, xb, kb, vb, wqb, wob,
            out_ref,
            x_buf, wq_buf, wo_buf, q_scr, o_scr, k_buf, v_buf,
            sem_x, sem_wq, sem_wo, sem_kv):
    w = pl.program_id(0)
    j = pl.program_id(1)

    def x_copy(src, i):
        return pltpu.make_async_copy(src, x_buf.at[i], sem_x.at[i])

    def wq_copy(src, i):
        return pltpu.make_async_copy(src, wq_buf.at[i], sem_wq.at[i])

    def wo_copy(src, i):
        return pltpu.make_async_copy(src, wo_buf.at[i], sem_wo.at[i])

    def kv_copies(k_src, v_src, batch, slot):
        return (pltpu.make_async_copy(k_src.at[batch], k_buf.at[slot], sem_kv.at[slot, 0]),
                pltpu.make_async_copy(v_src.at[batch], v_buf.at[slot], sem_kv.at[slot, 1]))

    def kv_start(item):
        slot = item % NB
        batch = item % B

        def start(k_src, v_src):
            for c in kv_copies(k_src, v_src, batch, slot):
                c.start()

        if isinstance(item, int):
            start(ka, va) if item < B else start(kb, vb)
        else:
            @pl.when(item < B)
            def _():
                start(ka, va)

            @pl.when(item >= B)
            def _():
                start(kb, vb)

    def kv_wait(item):
        slot = item % NB
        batch = item % B

        def wait(k_src, v_src):
            for c in kv_copies(k_src, v_src, batch, slot):
                c.wait()

        @pl.when(item < B)
        def _():
            wait(ka, va)

        @pl.when(item >= B)
        def _():
            wait(kb, vb)

    @pl.when(jnp.logical_and(w == 0, j == 0))
    def _():
        x_copy(xa, 0).start()
        wq_copy(wqa, 0).start()
        kv_start(0)
        wo_copy(woa, 0).start()
        for item in range(1, NB - 1):
            kv_start(item)

    @pl.when(jnp.logical_and(w == 0, j == 1))
    def _():
        x_copy(xb, 1).start()
        wq_copy(wqb, 1).start()
        wo_copy(wob, 1).start()

    @pl.when(j == 0)
    def _():
        @pl.when(w == 0)
        def _():
            x_copy(xa, 0).wait()
            wq_copy(wqa, 0).wait()

        @pl.when(w == 1)
        def _():
            x_copy(xb, 1).wait()
            wq_copy(wqb, 1).wait()

        def body(b, carry):
            q = jnp.dot(x_buf[w, b], wq_buf[w], preferred_element_type=jnp.float32)
            q_scr[b] = (q * Q_SCALE).astype(jnp.bfloat16)
            return carry

        lax.fori_loop(0, B, body, 0)

    @pl.when(j > 0)
    def _():
        b = j - 1
        item = w * B + b
        slot = item % NB

        @pl.when(item + (NB - 1) < NITEMS)
        def _():
            kv_start(item + (NB - 1))

        kv_wait(item)

        s_next = _qk(q_scr[b, :, 0:DH], k_buf[slot, 0])
        for h in range(H):
            s = s_next
            if h + 1 < H:
                s_next = _qk(q_scr[b, :, (h + 1) * DH:(h + 2) * DH], k_buf[slot, h + 1])
            o_scr[:, h * DH:(h + 1) * DH] = _softmax_pv(s, v_buf[slot, h])

        @pl.when(jnp.logical_and(w == 0, j == 1))
        def _():
            wo_copy(woa, 0).wait()

        @pl.when(jnp.logical_and(w == 1, j == 1))
        def _():
            wo_copy(wob, 1).wait()

        out = jnp.dot(o_scr[...], wo_buf[w], preferred_element_type=jnp.float32)
        out_ref[0] = out.astype(out_ref.dtype)


@jax.jit
def pallas_concat_heads__mha_block_cached__mha_block_cached__near_ridge_kernel(
    A_x: jax.Array,
    A_k_cache: jax.Array,
    A_v_cache: jax.Array,
    A_wq: jax.Array,
    A_wo: jax.Array,
    B_x: jax.Array,
    B_k_cache: jax.Array,
    B_v_cache: jax.Array,
    B_wq: jax.Array,
    B_wo: jax.Array,
):
    dt = A_x.dtype
    any_spec = pl.BlockSpec(memory_space=pl.ANY)
    return pl.pallas_call(
        _kernel,
        grid=(NBLK, B + 1),
        in_specs=[any_spec] * 10,
        out_specs=pl.BlockSpec((1, SQ, D), lambda w, j: (jnp.maximum(j - 1, 0), 0, w)),
        out_shape=jax.ShapeDtypeStruct((B, SQ, NBLK * D), dt),
        scratch_shapes=[
            pltpu.VMEM((NBLK, B, SQ, D), dt),
            pltpu.VMEM((NBLK, D, HD), dt),
            pltpu.VMEM((NBLK, HD, D), dt),
            pltpu.VMEM((B, SQ, HD), dt),
            pltpu.VMEM((SQ, HD), dt),
            pltpu.VMEM((NB, H, SK, DH), dt),
            pltpu.VMEM((NB, H, SK, DH), dt),
            pltpu.SemaphoreType.DMA((NBLK,)),
            pltpu.SemaphoreType.DMA((NBLK,)),
            pltpu.SemaphoreType.DMA((NBLK,)),
            pltpu.SemaphoreType.DMA((NB, 2)),
        ],
        compiler_params=pltpu.CompilerParams(
            dimension_semantics=("arbitrary", "arbitrary"),
            vmem_limit_bytes=110 * 1024 * 1024,
        ),
    )(A_x, A_k_cache, A_v_cache, A_wq, A_wo, B_x, B_k_cache, B_v_cache, B_wq, B_wo)
```

```python
import math

import jax
import jax.numpy as jnp
from jax import lax
import jax.experimental.pallas as pl
import jax.experimental.pallas.tpu as pltpu

B, SQ, D = 8, 144, 640
H, SK, DH = 32, 512, 128
HD = H * DH
NBLK = 2
NITEMS = NBLK * B
NB = 3
Q_LEAD = 5
NQ = Q_LEAD + 1
GH = 4
NG = H // GH
GW = GH * DH

Q_SCALE = (DH ** -0.5) * math.log2(math.e)


def _qk(q, k):
    return lax.dot_general(q, k, (((1,), (1,)), ((), ())),
                           preferred_element_type=jnp.float32)


def _softmax_pv(s, v):
    m = jnp.max(s, axis=-1, keepdims=True)
    p = jnp.exp2(s - m)
    l = jnp.sum(p, axis=-1, keepdims=True)
    o = jnp.dot(p.astype(jnp.bfloat16), v, preferred_element_type=jnp.float32)
    r = pl.reciprocal(l, approx=True)
    r = r * (2.0 - l * r)
    return (o * r).astype(jnp.bfloat16)


def _kernel(xa, ka, va, wqa, woa, xb, kb, vb, wqb, wob,
            out_ref,
            x_buf, wq_buf, wo_buf, q_scr, o_scr, k_buf, v_buf,
            sem_x, sem_wq, sem_wo, sem_kv):
    step = pl.program_id(0)

    def x_copy(src, blk):
        return pltpu.make_async_copy(src, x_buf.at[blk], sem_x.at[blk])

    def wq_copy(src, blk):
        return pltpu.make_async_copy(src, wq_buf.at[blk], sem_wq.at[blk])

    def wo_copy(src, blk):
        return pltpu.make_async_copy(src, wo_buf.at[blk], sem_wo.at[blk])

    def kv(item, op):
        slot = item % NB
        batch = item % B

        def go(k_src, v_src):
            getattr(pltpu.make_async_copy(k_src.at[batch], k_buf.at[slot],
                                          sem_kv.at[slot, 0]), op)()
            getattr(pltpu.make_async_copy(v_src.at[batch], v_buf.at[slot],
                                          sem_kv.at[slot, 1]), op)()

        if isinstance(item, int):
            if item < B:
                go(ka, va)
            else:
                go(kb, vb)
        else:
            @pl.when(item < B)
            def _():
                go(ka, va)

            @pl.when(item >= B)
            def _():
                go(kb, vb)

    def qproj_chunk(item, c):
        blk = item // B
        batch = item % B
        q = jnp.dot(x_buf[blk, batch], wq_buf[blk, :, c * GW:(c + 1) * GW],
                    preferred_element_type=jnp.float32)
        q_scr[item % NQ, :, c * GW:(c + 1) * GW] = (q * Q_SCALE).astype(q_scr.dtype)

    def attention(t, with_q):
        blk = t // B
        slot = t % NB
        qslot = t % NQ
        nxt = t + Q_LEAD

        def q_of(h):
            return q_scr[qslot, :, h * DH:(h + 1) * DH]

        def out_group(g):
            return jnp.dot(o_scr[:, g * GW:(g + 1) * GW],
                           wo_buf[blk, g * GW:(g + 1) * GW, :],
                           preferred_element_type=jnp.float32)

        s_cur = _qk(q_of(0), k_buf[slot, 0])
        s_nxt = _qk(q_of(1), k_buf[slot, 1])
        if with_q:
            qproj_chunk(nxt, 0)
        acc = None
        for h in range(H):
            o_scr[:, h * DH:(h + 1) * DH] = _softmax_pv(s_cur, v_buf[slot, h])
            s_cur = s_nxt
            if h + 2 < H:
                s_nxt = _qk(q_of(h + 2), k_buf[slot, h + 2])
            if h % GH == 0 and h > 0:
                part = out_group(h // GH - 1)
                acc = part if acc is None else acc + part
            if with_q and h % GH == 2 and h // GH + 1 < NG - 1:
                qproj_chunk(nxt, h // GH + 1)
        if with_q:
            qproj_chunk(nxt, NG - 1)
        acc = acc + out_group(NG - 1)
        out_ref[0] = acc.astype(out_ref.dtype)

    @pl.when(step == 0)
    def _():
        x_copy(xa, 0).start()
        wq_copy(wqa, 0).start()
        x_copy(xa, 0).wait()
        wq_copy(wqa, 0).wait()
        kv(0, "start")

        def body(item, carry):
            @pl.when(item == min(1, Q_LEAD - 1))
            def _():
                wo_copy(woa, 0).start()

            @pl.when(item == Q_LEAD - 1)
            def _():
                for nxt in range(1, NB - 1):
                    kv(nxt, "start")

            for c in range(NG):
                qproj_chunk(item, c)
            return carry

        lax.fori_loop(0, Q_LEAD, body, 0)

    @pl.when(step > 0)
    def _():
        t = step - 1

        @pl.when(t == B - Q_LEAD - (NB - 1))
        def _():
            x_copy(xb, 1).start()
            wq_copy(wqb, 1).start()

        @pl.when(t == B - (NB - 1))
        def _():
            wo_copy(wob, 1).start()

        @pl.when(t + (NB - 1) < NITEMS)
        def _():
            kv(t + (NB - 1), "start")

        @pl.when(t == B - Q_LEAD)
        def _():
            x_copy(xb, 1).wait()
            wq_copy(wqb, 1).wait()

        @pl.when(t == 0)
        def _():
            wo_copy(woa, 0).wait()

        @pl.when(t == B)
        def _():
            wo_copy(wob, 1).wait()

        kv(t, "wait")

        @pl.when(t + Q_LEAD < NITEMS)
        def _():
            attention(t, True)

        @pl.when(t + Q_LEAD >= NITEMS)
        def _():
            attention(t, False)


def _out_block(step):
    t = jnp.maximum(step - 1, 0)
    return (t % B, 0, t // B)


@jax.jit
def pallas_concat_heads__mha_block_cached__mha_block_cached__near_ridge_kernel(
    A_x: jax.Array,
    A_k_cache: jax.Array,
    A_v_cache: jax.Array,
    A_wq: jax.Array,
    A_wo: jax.Array,
    B_x: jax.Array,
    B_k_cache: jax.Array,
    B_v_cache: jax.Array,
    B_wq: jax.Array,
    B_wo: jax.Array,
):
    dt = A_x.dtype
    hbm = pl.BlockSpec(memory_space=pl.ANY)
    return pl.pallas_call(
        _kernel,
        grid=(NITEMS + 1,),
        in_specs=[hbm] * 10,
        out_specs=pl.BlockSpec((1, SQ, D), _out_block),
        out_shape=jax.ShapeDtypeStruct((B, SQ, NBLK * D), dt),
        scratch_shapes=[
            pltpu.VMEM((NBLK, B, SQ, D), dt),
            pltpu.VMEM((NBLK, D, HD), dt),
            pltpu.VMEM((NBLK, HD, D), dt),
            pltpu.VMEM((NQ, SQ, HD), dt),
            pltpu.VMEM((SQ, HD), dt),
            pltpu.VMEM((NB, H, SK, DH), dt),
            pltpu.VMEM((NB, H, SK, DH), dt),
            pltpu.SemaphoreType.DMA((NBLK,)),
            pltpu.SemaphoreType.DMA((NBLK,)),
            pltpu.SemaphoreType.DMA((NBLK,)),
            pltpu.SemaphoreType.DMA((NB, 2)),
        ],
        compiler_params=pltpu.CompilerParams(
            dimension_semantics=("arbitrary",),
            vmem_limit_bytes=100 * 1024 * 1024,
        ),
    )(A_x, A_k_cache, A_v_cache, A_wq, A_wo, B_x, B_k_cache, B_v_cache, B_wq, B_wo)
```
